```python
import os as _os
_os.environ.setdefault("JAX_PLATFORMS", "cpu")
import jax
import jax.numpy as jnp

def _softmax(x, axis=-1):
    return jax.nn.softmax(x, axis=axis)
def _gelu(x):
    return jax.nn.gelu(x, approximate=True)
def _silu(x):
    return jax.nn.silu(x)
def _sigmoid(x):
    return jax.nn.sigmoid(x)
def _layernorm(x, axis=-1, eps=1e-5):
    m = jnp.mean(x, axis=axis, keepdims=True)
    v = jnp.var(x, axis=axis, keepdims=True)
    return (x - m) / jnp.sqrt(v + eps)
def _scatter_add(tgt, idx, src, axis=0):
    return tgt.at[idx].add(src)
def _segment_sum(src, seg, n):
    return jax.ops.segment_sum(src, seg, n)
class _Rng:
    def __init__(self, key):
        self._k = key
    def _next(self):
        self._k, sub = jax.random.split(self._k)
        return sub
    def normal(self, shape):
        return jax.random.normal(self._next(), shape, dtype=jnp.bfloat16)
    def randint(self, lo, hi, shape):
        return jax.random.randint(self._next(), shape, lo, hi, dtype=jnp.int32)
    def uniform(self, shape, lo=0.0, hi=1.0):
        return jax.random.uniform(self._next(), shape, jnp.bfloat16, lo, hi)
    def permutation(self, n):
        return jax.random.permutation(self._next(), n)


kernel_name = 'standalone__gqa_block_cached__near_ridge'

def setup_inputs():
    _rng = _Rng(jax.random.key(int.from_bytes(__import__("os").urandom(4), "little")))
    _w = (lambda a: (lambda t: t.astype(jnp.bfloat16) if jnp.issubdtype(t.dtype, jnp.floating) else t)(jnp.asarray(a)))
    B, Sq, D = 16, 128, 576
    Hq, Hkv, Sk, Dh = 32, 16, 1024, 128
    assert Hq % Hkv == 0, (Hq, Hkv)
    return {
        "x": _w((lambda *s: _rng.normal(s) * 0.8)(B, Sq, D)),
        "k_cache": _w((lambda *s: _rng.normal(s) * 0.8)(B, Hkv, Sk, Dh)),
        "v_cache": _w((lambda *s: _rng.normal(s) * 0.05)(B, Hkv, Sk, Dh)),
        "wq": _w((lambda *s: _rng.normal(s) * 0.8)(D, Hq * Dh) * (D ** -0.5)),
        "wo": _w((lambda *s: _rng.normal(s) * 0.05)(Hq * Dh, D) * ((Hq * Dh) ** -0.5)),
    }

def reference(x, k_cache, v_cache, wq, wo):
    B, Sq, D = x.shape
    Hq, Dh = 32, 128
    Hkv = k_cache.shape[1]
    rep = Hq // Hkv
    q = (lambda x, *d: x.transpose(*d))((x @ wq).reshape(B, Sq, Hq, Dh), 0, 2, 1, 3)
    k = jnp.repeat(k_cache, rep, axis=1)
    v = jnp.repeat(v_cache, rep, axis=1)
    scores = jnp.einsum("bhqd,bhkd->bhqk", q, k) * (Dh ** -0.5)
    p = _softmax(scores, axis=-1)
    o = jnp.einsum("bhqk,bhkd->bhqd", p, v)
    return (lambda x, *d: x.transpose(*d))(o, 0, 2, 1, 3).reshape(B, Sq, Hq * Dh) @ wo
```

```python
import jax
import jax.numpy as jnp
import jax.experimental.pallas as pl
import jax.experimental.pallas.tpu as pltpu

LOG2E = 1.4426950408889634
NT = (((1,), (1,)), ((), ()))
F32, BF16 = jnp.float32, jnp.bfloat16

def make(vmem=100, rc=32, order="ZCAD", bpos=0, flags=None, nob=False, dcat=False, qdbl=True, split=False):
    bb = 4
    c = (128 ** -0.5) * LOG2E
    NJ = 32

    def kern(xt_hbm, k_hbm, v_hbm, wq_hbm, wot_hbm, o_hbm,
             xt_v, x_s, wq_s, wo_s, kbuf, vbuf, q0, q1, s0, s1, p0, p1, l0, l1, o0, o1, acc_s, ost,
             xsem, wqsem, wosem, ksem, vsem, osem):
        S_ = (s0, s1); P_ = (p0, p1); L_ = (l0, l1); Q_ = (q0, q1) if qdbl else (q0, q0); O_ = (o0, o1)

        def x_copy(g):
            return pltpu.make_async_copy(xt_hbm.at[pl.ds(g * bb, bb)], xt_v, xsem)
        def wq_copy(j):
            return pltpu.make_async_copy(wq_hbm.at[:, pl.ds(pl.multiple_of(j * 512, 512), 512)], wq_s.at[j], wqsem)
        def wo_copy(j):
            return pltpu.make_async_copy(wot_hbm.at[:, pl.ds(pl.multiple_of(j * 512, 512), 512)], wo_s.at[j], wosem)
        def k_copy(j):
            g = j >> 3; h = (j & 7) * 2
            return pltpu.make_async_copy(k_hbm.at[pl.ds(g * bb, bb), pl.ds(h, 2)], kbuf.at[j & 1], ksem.at[j & 1])
        def v_copy(j):
            g = j >> 3; h = (j & 7) * 2
            return pltpu.make_async_copy(v_hbm.at[pl.ds(g * bb, bb), pl.ds(h, 2)], vbuf.at[j & 1], vsem.at[j & 1])
        def o_copy(g):
            return pltpu.make_async_copy(ost, o_hbm.at[pl.ds(g * bb, bb)], osem)

        def transpose_x():
            for i in range(bb):
                xp = jnp.concatenate([xt_v[i], jnp.zeros((64, 128), BF16)], axis=0)
                x_s[i * 128:(i + 1) * 128, :] = xp.T[:, :576]

        def stage_z(j, par):
            q = jnp.dot(x_s[...], wq_s[j & 7, :, par * 256:(par + 1) * 256], preferred_element_type=F32)
            q = (q * c).astype(BF16)
            for i in range(bb):
                for jj in range(2):
                    Q_[par][i, jj * 128:(jj + 1) * 128, :] = q[i * 128:(i + 1) * 128, jj * 128:(jj + 1) * 128]

        def stage_a(j, i, par):
            S_[par][i] = jax.lax.dot_general(Q_[par][i], kbuf[j & 1, i, par], NT, preferred_element_type=F32)

        def stage_b(i, par):
            for r in range(0, 256, rc):
                s = S_[par][i, r:r + rc, :]
                m = jnp.max(s, axis=-1, keepdims=True)
                p = jnp.exp2(s - m)
                l = jnp.sum(p, axis=-1, keepdims=True)
                P_[par][i, r:r + rc, :] = p.astype(BF16)
                L_[par][i, r:r + rc, :] = jnp.broadcast_to(1.0 / l, (rc, 128))

        def stage_c(jv, i, par):
            o = jnp.dot(P_[par][i], vbuf[jv & 1, i, par], preferred_element_type=F32)
            o = (o * L_[par][i]).astype(BF16)
            return jnp.concatenate([o[:128], o[128:]], axis=1)

        def stage_d(jv, os_, par):
            oall = jnp.concatenate(os_, axis=0)
            r = jax.lax.dot_general(wo_s[jv & 7, :, par * 256:(par + 1) * 256], oall, NT, preferred_element_type=F32)
            acc_s[...] += r

        def substep(j, par, za, b, cd):
            os_ = None
            for k, ch in enumerate(order):
                if b and k == bpos:
                    for i in range(bb): stage_b(i, 1 - par)
                if ch == "Z" and za: stage_z(j, par)
                if ch == "A" and za:
                    for i in range(bb): stage_a(j, i, par)
                if ch == "C" and cd:
                    os_ = [stage_c(j - 1, i, par) for i in range(bb)]
                    if dcat:
                        for i in range(bb): O_[par][i * 128:(i + 1) * 128, :] = os_[i]
                if ch == "D" and cd:
                    if not dcat:
                        stage_d(j - 1, os_, par)
                    elif par == 1:
                        oall = jnp.concatenate([o0[...], o1[...]], axis=1)
                        acc_s[...] += jax.lax.dot_general(wo_s[(j - 1) & 7], oall, NT, preferred_element_type=F32)

        def write_out(g):
            for i in range(bb):
                ost[i] = acc_s[:, i * 128:(i + 1) * 128].astype(ost.dtype)
            o_copy(g).start()

        x_copy(0).start(); wq_copy(0).start(); k_copy(0).start()
        acc_s[...] = jnp.zeros_like(acc_s)
        x_copy(0).wait()
        transpose_x()
        wq_copy(0).wait()
        k_copy(0).wait()
        wq_copy(1).start(); k_copy(1).start(); v_copy(0).start(); wo_copy(0).start()
        substep(0, 0, True, False, False)
        substep(0, 1, True, True, False)

        def pre(j):
            k_copy(j).wait()
            v_copy(j - 1).wait()

            @pl.when(j < 8)
            def _():
                wq_copy(j).wait()
                wo_copy(j - 1).wait()
                wo_copy(j).start()

                @pl.when(j < 7)
                def _():
                    wq_copy(j + 1).start()

            @pl.when(j == 8)
            def _():
                wo_copy(7).wait()

            @pl.when(j < NJ - 1)
            def _():
                k_copy(j + 1).start()
            v_copy(j).start()

            @pl.when((j & 7) == 0)
            def _():
                x_copy(j >> 3).wait()
                transpose_x()

            @pl.when((j & 7) == 4)
            def _():
                @pl.when(j < NJ - 8)
                def _():
                    x_copy((j >> 3) + 1).start()

        def post(j):
            @pl.when((j & 7) == 0)
            def _():
                @pl.when(j > 8)
                def _():
                    o_copy((j >> 3) - 2).wait()
                write_out((j >> 3) - 1)
                acc_s[...] = jnp.zeros_like(acc_s)

        if split:
            def body(t, carry):
                j = t >> 1

                @pl.when((t & 1) == 0)
                def _():
                    pre(j)
                    substep(j, 0, True, not nob, True)

                @pl.when((t & 1) == 1)
                def _():
                    substep(j, 1, True, not nob, True)
                    post(j)
                return carry
            jax.lax.fori_loop(2, 2 * NJ, body, 0)
        else:
            def body(j, carry):
                pre(j)
                substep(j, 0, True, not nob, True)
                substep(j, 1, True, not nob, True)
                post(j)
                return carry
            jax.lax.fori_loop(1, NJ, body, 0)
        v_copy(NJ - 1).wait()
        substep(NJ, 0, False, True, True)
        substep(NJ, 1, False, False, True)
        o_copy(2).wait()
        write_out(3)
        o_copy(3).wait()

    @jax.jit
    def f(x, k_cache, v_cache, wq, wo):
        B, Sq, D = x.shape
        Hkv, Sk, Dh = k_cache.shape[1:]
        xt = jnp.transpose(x, (0, 2, 1))
        wot = wo.T
        anyspec = pl.BlockSpec(memory_space=pltpu.HBM)
        out = pl.pallas_call(
            kern,
            in_specs=[anyspec] * 5,
            out_specs=anyspec,
            out_shape=jax.ShapeDtypeStruct((B, D, Sq), x.dtype),
            scratch_shapes=[
                pltpu.VMEM((bb, D, Sq), BF16),
                pltpu.VMEM((bb * Sq, D), BF16),
                pltpu.VMEM((8, D, 512), BF16),
                pltpu.VMEM((8, D, 512), BF16),
                pltpu.VMEM((2, bb, 2, Sk, Dh), BF16),
                pltpu.VMEM((2, bb, 2, Sk, Dh), BF16),
                pltpu.VMEM((bb, 256, 128), BF16), pltpu.VMEM((bb, 256, 128), BF16),
                pltpu.VMEM((bb, 256, Sk), F32), pltpu.VMEM((bb, 256, Sk), F32),
                pltpu.VMEM((bb, 256, Sk), BF16), pltpu.VMEM((bb, 256, Sk), BF16),
                pltpu.VMEM((bb, 256, 128), F32), pltpu.VMEM((bb, 256, 128), F32),
                pltpu.VMEM((bb * Sq, 256), BF16), pltpu.VMEM((bb * Sq, 256), BF16),
                pltpu.VMEM((D, bb * Sq), F32),
                pltpu.VMEM((bb, D, Sq), BF16),
                pltpu.SemaphoreType.DMA(()), pltpu.SemaphoreType.DMA(()), pltpu.SemaphoreType.DMA(()),
                pltpu.SemaphoreType.DMA((2,)), pltpu.SemaphoreType.DMA((2,)), pltpu.SemaphoreType.DMA(()),
            ],
            compiler_params=pltpu.CompilerParams(vmem_limit_bytes=vmem * 1024 * 1024, flags=flags),
        )(xt, k_cache, v_cache, wq, wot)
        return jnp.transpose(out, (0, 2, 1))
    return f


_impl = make(split=True, rc=64, flags={"XLA_TPU_EVENLY_DISTRIBUTE_CRITICAL_NODES": True})


@jax.jit
def pallas_standalone__gqa_block_cached__near_ridge_kernel(x, k_cache, v_cache, wq, wo):
    return _impl(x, k_cache, v_cache, wq, wo)
```

```python
import jax
import jax.numpy as jnp
import jax.experimental.pallas as pl
import jax.experimental.pallas.tpu as pltpu

B, SQ, D = 16, 128, 576
HQ, HKV, SK, DH = 32, 16, 1024, 128
REP = HQ // HKV
BB = 8
NG = B // BB
NU = NG * HKV
HSH = HKV.bit_length() - 1
W = REP * DH
NCH = 2
CB = BB // NCH
QSCALE = (DH ** -0.5) * 1.4426950408889634
NT = (((1,), (1,)), ((), ()))
F32, BF16 = jnp.float32, jnp.bfloat16


def _kernel(xt_hbm, k_hbm, v_hbm, wq_hbm, wot_hbm, o_hbm,
            xt_v, x_s, wq_s, wo_s, k0, k1, v0, v1, q0, q1, s0, s1, p0, p1, l0, l1, acc_s, ost,
            xsem, wqsem, wosem, ksem, vsem, osem):
    K_, V_, Q_, S_, P_, L_ = (k0, k1), (v0, v1), (q0, q1), (s0, s1), (p0, p1), (l0, l1)

    def x_copy(g):
        return pltpu.make_async_copy(xt_hbm.at[pl.ds(g * BB, BB)], xt_v, xsem)

    def w_copy(hbm, buf, sem, h):
        return pltpu.make_async_copy(hbm.at[:, pl.ds(pl.multiple_of(h * W, W), W)], buf.at[h], sem)

    def kv_copy(hbm, buf, sem, u):
        return pltpu.make_async_copy(hbm.at[pl.ds((u >> HSH) * BB, BB), u & (HKV - 1)], buf, sem)

    wq_copy = lambda h: w_copy(wq_hbm, wq_s, wqsem, h)
    wo_copy = lambda h: w_copy(wot_hbm, wo_s, wosem, h)
    k_copy = lambda u, par: kv_copy(k_hbm, K_[par], ksem.at[par], u)
    v_copy = lambda u, par: kv_copy(v_hbm, V_[par], vsem.at[par], u)

    def o_copy(g, n, sem):
        return pltpu.make_async_copy(ost.at[pl.ds(n * CB, CB)], o_hbm.at[pl.ds(g * BB + n * CB, CB)], sem)

    def transpose_x():
        for i in range(BB):
            xp = jnp.concatenate([xt_v[i], jnp.zeros((640 - D, SQ), BF16)], axis=0)
            x_s[i * SQ:(i + 1) * SQ, :] = xp.T[:, :D]

    def project_q(x, h, par, i0, nb):
        q = (jnp.dot(x, wq_s[h], preferred_element_type=F32) * QSCALE).astype(BF16)
        for i in range(nb):
            for r in range(REP):
                Q_[par][i0 + i, r * SQ:(r + 1) * SQ, :] = q[i * SQ:(i + 1) * SQ, r * DH:(r + 1) * DH]

    def scores(par, i):
        S_[par][i] = jax.lax.dot_general(Q_[par][i], K_[par][i], NT, preferred_element_type=F32)

    def softmax(par):
        for i in range(BB):
            s = S_[par][i]
            p = jnp.exp2(s - jnp.max(s, axis=-1, keepdims=True))
            P_[par][i] = p.astype(BF16)
            L_[par][i] = jnp.broadcast_to(1.0 / jnp.sum(p, axis=-1, keepdims=True), (REP * SQ, DH))

    def attend(par, i):
        o = jnp.dot(P_[par][i], V_[par][i], preferred_element_type=F32)
        o = (o * L_[par][i]).astype(BF16)
        return jnp.concatenate([o[r * SQ:(r + 1) * SQ] for r in range(REP)], axis=1)

    def out_proj(h, outs):
        return jax.lax.dot_general(wo_s[h], jnp.concatenate(outs, axis=0), NT, preferred_element_type=F32)

    def step(t, par, z=True, a=True, cd=True):
        softmax(1 - par)
        if cd:
            outs = [attend(par, i) for i in range(BB)]
        if z:
            project_q(x_s[...], (t + 1) & (HKV - 1), 1 - par, 0, BB)
        if cd:
            h = (t - 2) & (HKV - 1)
            r = out_proj(h, outs)
            for n in range(NCH):
                acc_s[n] = jnp.where(h == 0, 0.0, acc_s[n]) + r[:, n * CB * SQ:(n + 1) * CB * SQ]
        if a:
            for i in range(BB):
                scores(par, i)

    def stream(t, par):
        k_copy(t, par).wait()
        v_copy(t - 2, par).wait()
        v_copy(t - 1, 1 - par).start()
        k_copy(t + 1, 1 - par).start()

        @pl.when(t < HKV + 2)
        def _():
            @pl.when(t < HKV - 1)
            def _():
                wq_copy(t + 1).wait()
            wo_copy(t - 2).wait()

            @pl.when(t < HKV - 2)
            def _():
                wq_copy(t + 2).start()

            @pl.when(t < HKV + 1)
            def _():
                wo_copy(t - 1).start()

    def z_rolled(h, par):
        def body(n, c):
            project_q(x_s[pl.ds(pl.multiple_of(n * CB * SQ, CB * SQ), CB * SQ), :], h, par, n * CB, CB)
            return c
        jax.lax.fori_loop(0, NCH, body, 0)

    def a_rolled(par):
        def body(n, c):
            scores(par, 2 * n)
            scores(par, 2 * n + 1)
            return c
        jax.lax.fori_loop(0, BB // 2, body, 0)

    x_copy(0).start()
    wq_copy(0).start()
    k_copy(0, 0).start()
    acc_s[...] = jnp.zeros_like(acc_s)
    x_copy(0).wait()
    transpose_x()
    wq_copy(0).wait()
    wq_copy(1).start()
    k_copy(1, 1).start()
    z_rolled(0, 0)
    wq_copy(1).wait()
    k_copy(0, 0).wait()
    wq_copy(2).start()
    v_copy(0, 0).start()
    wo_copy(0).start()
    z_rolled(1, 1)
    a_rolled(0)
    wq_copy(2).wait()
    k_copy(1, 1).wait()
    wq_copy(3).start()
    k_copy(2, 0).start()
    step(1, 1, cd=False)

    def body(t, c):
        @pl.when((t & 1) == 0)
        def _():
            stream(t, 0)

            @pl.when(jnp.logical_and((t & (HKV - 1)) == HKV // 2, t < NU - HKV))
            def _():
                x_copy((t >> HSH) + 1).start()
            step(t, 0)

        @pl.when((t & 1) == 1)
        def _():
            stream(t, 1)

            @pl.when((t & (HKV - 1)) == HKV - 1)
            def _():
                x_copy((t + 1) >> HSH).wait()
                transpose_x()
            step(t, 1)

            @pl.when((t & (HKV - 1)) == 1)
            def _():
                g = (t >> HSH) - 1

                @pl.when(g > 0)
                def _():
                    for n in range(NCH):
                        o_copy(g - 1, n, osem.at[n]).wait()
                for i in range(BB):
                    ost[i] = acc_s[i // CB, :, (i % CB) * SQ:(i % CB + 1) * SQ].astype(ost.dtype)
                for n in range(NCH):
                    o_copy(g, n, osem.at[n]).start()
        return c
    jax.lax.fori_loop(2, NU - 1, body, 0)

    k_copy(NU - 1, 1).wait()
    v_copy(NU - 3, 1).wait()
    v_copy(NU - 2, 0).start()
    step(NU - 1, 1, z=False)
    v_copy(NU - 2, 0).wait()
    v_copy(NU - 1, 1).start()
    step(NU, 0, z=False, a=False)
    v_copy(NU - 1, 1).wait()
    for n in range(NCH):
        o_copy(NG - 2, n, osem.at[n]).wait()
    for n in range(NCH):
        r = out_proj(HKV - 1, [attend(1, n * CB + i) for i in range(CB)]) + acc_s[n]
        for i in range(CB):
            ost[n * CB + i] = r[:, i * SQ:(i + 1) * SQ].astype(ost.dtype)
        o_copy(NG - 1, n, osem.at[n]).start()
    for n in range(NCH):
        o_copy(NG - 1, n, osem.at[n]).wait()


@jax.jit
def pallas_standalone__gqa_block_cached__near_ridge_kernel(x, k_cache, v_cache, wq, wo):
    vm = pltpu.VMEM
    dma = pltpu.SemaphoreType.DMA
    hbm = pl.BlockSpec(memory_space=pltpu.HBM)
    out_t = pl.pallas_call(
        _kernel,
        in_specs=[hbm] * 5,
        out_specs=hbm,
        out_shape=jax.ShapeDtypeStruct((B, D, SQ), x.dtype),
        scratch_shapes=[
            vm((BB, D, SQ), BF16),
            vm((BB * SQ, D), BF16),
            vm((HKV, D, W), BF16),
            vm((HKV, D, W), BF16),
            *[vm((BB, SK, DH), BF16)] * 4,
            *[vm((BB, REP * SQ, DH), BF16)] * 2,
            *[vm((BB, REP * SQ, SK), F32)] * 2,
            *[vm((BB, REP * SQ, SK), BF16)] * 2,
            *[vm((BB, REP * SQ, DH), F32)] * 2,
            vm((NCH, D, CB * SQ), F32),
            vm((BB, D, SQ), BF16),
            dma(()), dma(()), dma(()), dma((2,)), dma((2,)), dma((NCH,)),
        ],
        compiler_params=pltpu.CompilerParams(
            vmem_limit_bytes=100 * 1024 * 1024,
            disable_bounds_checks=True,
            flags={"XLA_TPU_EVENLY_DISTRIBUTE_CRITICAL_NODES": True},
        ),
    )(jnp.transpose(x, (0, 2, 1)), k_cache, v_cache, wq, wo.T)
    return jnp.transpose(out_t, (0, 2, 1))
```

```python
import jax
import jax.numpy as jnp
import jax.experimental.pallas as pl
import jax.experimental.pallas.tpu as pltpu

B, SQ, D = 16, 128, 576
HQ, HKV, SK, DH = 32, 16, 1024, 128
REP = HQ // HKV
BB = 8
NG = B // BB
NU = NG * HKV
HSH = HKV.bit_length() - 1
W = REP * DH
NCH = 2
CB = BB // NCH
QSCALE = (DH ** -0.5) * 1.4426950408889634
AC = 4
NT = (((1,), (1,)), ((), ()))
F32, BF16 = jnp.float32, jnp.bfloat16
assert NG == 2 and HKV == 1 << HSH


def _kernel(xt_hbm, k_hbm, v_hbm, wq_hbm, wot_hbm, o_hbm,
            xt_v, x_s, wq_s, wo_s, k0, k1, v0, v1, q_s, s0, s1, p0, p1, l0, l1, acc_s, ost,
            xsem, wqsem, wosem, ksem, vsem, osem):
    K_, V_, S_, P_, L_ = (k0, k1), (v0, v1), (s0, s1), (p0, p1), (l0, l1)

    def x_copy(g):
        return pltpu.make_async_copy(xt_hbm.at[pl.ds(g * BB, BB)], xt_v, xsem)

    def w_copy(hbm, buf, sem, h):
        return pltpu.make_async_copy(hbm.at[:, pl.ds(pl.multiple_of(h * W, W), W)], buf.at[h], sem)

    def kv_copy(hbm, buf, sem, u):
        return pltpu.make_async_copy(hbm.at[pl.ds((u >> HSH) * BB, BB), u & (HKV - 1)], buf, sem)

    wq_copy = lambda h: w_copy(wq_hbm, wq_s, wqsem.at[h & 3], h)
    wo_copy = lambda h: w_copy(wot_hbm, wo_s, wosem, h)
    k_copy = lambda u, par: kv_copy(k_hbm, K_[par], ksem.at[par], u)
    v_copy = lambda u, par: kv_copy(v_hbm, V_[par], vsem.at[par], u)

    def o_copy(g, n, sem):
        return pltpu.make_async_copy(ost.at[pl.ds(n * CB, CB)], o_hbm.at[pl.ds(g * BB + n * CB, CB)], sem)

    def transpose_x():
        for i in range(BB):
            xp = jnp.concatenate([xt_v[i], jnp.zeros((640 - D, SQ), BF16)], axis=0)
            x_s[i * SQ:(i + 1) * SQ, :] = xp.T[:, :D]

    def project_q(u):
        q = (jnp.dot(x_s[...], wq_s[u & (HKV - 1)], preferred_element_type=F32) * QSCALE).astype(BF16)
        for i in range(BB):
            for r in range(REP):
                q_s[u & 3, i, r * SQ:(r + 1) * SQ, :] = q[i * SQ:(i + 1) * SQ, r * DH:(r + 1) * DH]

    def scores(t, par, i):
        S_[par][i] = jax.lax.dot_general(q_s[t & 3, i], K_[par][i], NT, preferred_element_type=F32)

    def softmax(par):
        for i in range(BB):
            s = S_[par][i]
            p = jnp.exp2(s - jnp.max(s, axis=-1, keepdims=True))
            P_[par][i] = p.astype(BF16)
            L_[par][i] = jnp.broadcast_to(1.0 / jnp.sum(p, axis=-1, keepdims=True), (REP * SQ, DH))

    def attend(par, i):
        o = jnp.dot(P_[par][i], V_[par][i], preferred_element_type=F32)
        o = (o * L_[par][i]).astype(BF16)
        return jnp.concatenate([o[r * SQ:(r + 1) * SQ] for r in range(REP)], axis=1)

    def out_proj(h, outs):
        return jax.lax.dot_general(wo_s[h], jnp.concatenate(outs, axis=0), NT, preferred_element_type=F32)

    def step(t, par, z=True, a=True, cd=True, zt=None):
        softmax(1 - par)
        if cd:
            outs = [attend(par, i) for i in range(BB)]
        if z:
            project_q(zt)
        if cd:
            h = (t - 2) & (HKV - 1)
            r = out_proj(h, outs)
            for n in range(NCH):
                acc_s[n] = jnp.where(h == 0, 0.0, acc_s[n]) + r[:, n * CB * SQ:(n + 1) * CB * SQ]
        if a:
            for i in range(BB):
                scores(t, par, i)

    def stream(t, par, guard_k=False):
        k_copy(t, par).wait()
        v_copy(t - 2, par).wait()
        v_copy(t - 1, 1 - par).start()
        if guard_k:
            @pl.when(t < NU - 1)
            def _():
                k_copy(t + 1, 1 - par).start()
        else:
            k_copy(t + 1, 1 - par).start()

        @pl.when(t < HKV + 2)
        def _():
            @pl.when(t < HKV - 2)
            def _():
                wq_copy(t + 2).wait()
            wo_copy(t - 2).wait()

            @pl.when(t < HKV - 3)
            def _():
                wq_copy(t + 3).start()

            @pl.when(t < HKV + 1)
            def _():
                wo_copy(t - 1).start()

    x_copy(0).start()
    wq_copy(0).start()
    acc_s[...] = jnp.zeros_like(acc_s)
    x_copy(0).wait()
    for h in range(1, NG + 1):
        wq_copy(h).start()
    k_copy(0, 0).start()
    wq_copy(NG + 1).start()
    k_copy(1, 1).start()
    transpose_x()

    def z_body(u, c):
        wq_copy(u).wait()
        project_q(u)
        return c
    jax.lax.fori_loop(0, NG + 1, z_body, 0)
    k_copy(0, 0).wait()
    v_copy(0, 0).start()
    wo_copy(0).start()

    def a_body(n, c):
        for i in range(AC):
            scores(0, 0, n * AC + i)
        return c
    jax.lax.fori_loop(0, BB // AC, a_body, 0)
    wq_copy(NG + 1).wait()
    k_copy(1, 1).wait()
    wq_copy(NG + 2).start()
    k_copy(2, 0).start()
    step(1, 1, cd=False, zt=NG + 1)

    def body(t, c):
        zt = t + NG - (t >> HSH)
        last = (t & (HKV - 1)) == HKV - 1

        @pl.when((t & 1) == 0)
        def _():
            stream(t, 0)

            @pl.when(jnp.logical_and((t & (HKV - 1)) == HKV // 2, t < NU - HKV))
            def _():
                x_copy((t >> HSH) + 1).start()

            @pl.when((zt & (HKV - 1)) == 0)
            def _():
                x_copy(zt >> HSH).wait()
                transpose_x()
            step(t, 0, zt=zt)

        @pl.when(jnp.logical_and((t & 1) == 1, jnp.logical_not(last)))
        def _():
            stream(t, 1)
            step(t, 1, zt=zt)

            @pl.when((t & (HKV - 1)) == 1)
            def _():
                g = (t >> HSH) - 1
                for i in range(BB):
                    ost[i] = acc_s[i // CB, :, (i % CB) * SQ:(i % CB + 1) * SQ].astype(ost.dtype)
                for n in range(NCH):
                    o_copy(g, n, osem.at[n]).start()

        @pl.when(last)
        def _():
            stream(t, 1, guard_k=True)
            step(t, 1, z=False)
        return c
    jax.lax.fori_loop(2, NU, body, 0)

    v_copy(NU - 2, 0).wait()
    v_copy(NU - 1, 1).start()
    step(NU, 0, z=False, a=False)
    v_copy(NU - 1, 1).wait()
    for n in range(NCH):
        o_copy(NG - 2, n, osem.at[n]).wait()
    for n in range(NCH):
        r = out_proj(HKV - 1, [attend(1, n * CB + i) for i in range(CB)]) + acc_s[n]
        for i in range(CB):
            ost[n * CB + i] = r[:, i * SQ:(i + 1) * SQ].astype(ost.dtype)
        o_copy(NG - 1, n, osem.at[n]).start()
    for n in range(NCH):
        o_copy(NG - 1, n, osem.at[n]).wait()


@jax.jit
def pallas_standalone__gqa_block_cached__near_ridge_kernel(x, k_cache, v_cache, wq, wo):
    vm = pltpu.VMEM
    dma = pltpu.SemaphoreType.DMA
    hbm = pl.BlockSpec(memory_space=pltpu.HBM)
    out_t = pl.pallas_call(
        _kernel,
        in_specs=[hbm] * 5,
        out_specs=hbm,
        out_shape=jax.ShapeDtypeStruct((B, D, SQ), x.dtype),
        scratch_shapes=[
            vm((BB, D, SQ), BF16),
            vm((BB * SQ, D), BF16),
            vm((HKV, D, W), BF16),
            vm((HKV, D, W), BF16),
            *[vm((BB, SK, DH), BF16)] * 4,
            vm((4, BB, REP * SQ, DH), BF16),
            *[vm((BB, REP * SQ, SK), F32)] * 2,
            *[vm((BB, REP * SQ, SK), BF16)] * 2,
            *[vm((BB, REP * SQ, DH), F32)] * 2,
            vm((NCH, D, CB * SQ), F32),
            vm((BB, D, SQ), BF16),
            dma(()), dma((4,)), dma(()), dma((2,)), dma((2,)), dma((NCH,)),
        ],
        compiler_params=pltpu.CompilerParams(
            vmem_limit_bytes=100 * 1024 * 1024,
            disable_bounds_checks=True,
            flags={"XLA_TPU_EVENLY_DISTRIBUTE_CRITICAL_NODES": True},
        ),
    )(jnp.transpose(x, (0, 2, 1)), k_cache, v_cache, wq, wo.T)
    return jnp.transpose(out_t, (0, 2, 1))
```

```python
import jax
import jax.numpy as jnp
import jax.experimental.pallas as pl
import jax.experimental.pallas.tpu as pltpu

B, SQ, D = 16, 128, 576
HQ, HKV, SK, DH = 32, 16, 1024, 128
REP = HQ // HKV
BB = 8
NG = B // BB
NU = NG * HKV
HSH = HKV.bit_length() - 1
W = REP * DH
NCH = 2
CB = BB // NCH
QSCALE = (DH ** -0.5) * 1.4426950408889634
AC = 4
NT = (((1,), (1,)), ((), ()))
F32, BF16 = jnp.float32, jnp.bfloat16
assert NG == 2 and HKV == 1 << HSH


def _kernel(xt_hbm, k_hbm, v_hbm, wq_hbm, wot_hbm, o_hbm,
            xt_v, x_s, wq_s, wo_s, k0, k1, v0, v1, q_s, s0, s1, p0, p1, l0, l1, acc_s, ost,
            xsem, wqsem, wosem, ksem, vsem, osem):
    K_, V_, S_, P_, L_ = (k0, k1), (v0, v1), (s0, s1), (p0, p1), (l0, l1)

    def x_copy(g):
        return pltpu.make_async_copy(xt_hbm.at[pl.ds(g * BB, BB)], xt_v, xsem)

    def w_copy(hbm, buf, sem, h):
        return pltpu.make_async_copy(hbm.at[:, pl.ds(pl.multiple_of(h * W, W), W)], buf.at[h], sem)

    def kv_copy(hbm, buf, sem, u):
        return pltpu.make_async_copy(hbm.at[pl.ds((u >> HSH) * BB, BB), u & (HKV - 1)], buf, sem)

    wq_copy = lambda h: w_copy(wq_hbm, wq_s, wqsem.at[h & 3], h)
    wo_copy = lambda h: w_copy(wot_hbm, wo_s, wosem, h)
    k_copy = lambda u, par: kv_copy(k_hbm, K_[par], ksem.at[par], u)
    v_copy = lambda u, par: kv_copy(v_hbm, V_[par], vsem.at[par], u)

    def o_copy(g, n, sem):
        return pltpu.make_async_copy(ost.at[pl.ds(n * CB, CB)], o_hbm.at[pl.ds(g * BB + n * CB, CB)], sem)

    def transpose_x():
        for i in range(BB):
            xp = jnp.concatenate([xt_v[i], jnp.zeros((640 - D, SQ), BF16)], axis=0)
            x_s[i * SQ:(i + 1) * SQ, :] = xp.T[:, :D]

    def project_q(u):
        q = (jnp.dot(x_s[...], wq_s[u & (HKV - 1)], preferred_element_type=F32) * QSCALE).astype(BF16)
        for i in range(BB):
            for r in range(REP):
                q_s[u & 3, i, r * SQ:(r + 1) * SQ, :] = q[i * SQ:(i + 1) * SQ, r * DH:(r + 1) * DH]

    def scores(t, par, i):
        S_[par][i] = jax.lax.dot_general(q_s[t & 3, i], K_[par][i], NT, preferred_element_type=F32)

    def softmax(par):
        for i in range(BB):
            s = S_[par][i]
            p = jnp.exp2(s - jnp.max(s, axis=-1, keepdims=True))
            P_[par][i] = p.astype(BF16)
            L_[par][i] = jnp.broadcast_to(1.0 / jnp.sum(p, axis=-1, keepdims=True), (REP * SQ, DH))

    def attend(par, i):
        o = jnp.dot(P_[par][i], V_[par][i], preferred_element_type=F32)
        o = (o * L_[par][i]).astype(BF16)
        return jnp.concatenate([o[r * SQ:(r + 1) * SQ] for r in range(REP)], axis=1)

    def out_proj(h, outs):
        return jax.lax.dot_general(wo_s[h], jnp.concatenate(outs, axis=0), NT, preferred_element_type=F32)

    def step(t, par, z=True, a=True, cd=True, zt=None):
        softmax(1 - par)
        if cd:
            outs = [attend(par, i) for i in range(BB)]
        if z:
            project_q(zt)
        if cd:
            h = (t - 2) & (HKV - 1)
            r = out_proj(h, outs)
            for n in range(NCH):
                acc_s[n] = jnp.where(h == 0, 0.0, acc_s[n]) + r[:, n * CB * SQ:(n + 1) * CB * SQ]
        if a:
            for i in range(BB):
                scores(t, par, i)

    def stream(t, par, guard_k=False):
        k_copy(t, par).wait()
        v_copy(t - 2, par).wait()
        v_copy(t - 1, 1 - par).start()
        if guard_k:
            @pl.when(t < NU - 1)
            def _():
                k_copy(t + 1, 1 - par).start()
        else:
            k_copy(t + 1, 1 - par).start()

        @pl.when(t < HKV + 2)
        def _():
            @pl.when(t < HKV - 2)
            def _():
                wq_copy(t + 2).wait()
            wo_copy(t - 2).wait()

            @pl.when(t < HKV - 3)
            def _():
                wq_copy(t + 3).start()

            @pl.when(t < HKV + 1)
            def _():
                wo_copy(t - 1).start()

    x_copy(0).start()
    wq_copy(0).start()
    acc_s[...] = jnp.zeros_like(acc_s)
    x_copy(0).wait()
    for h in range(1, NG + 1):
        wq_copy(h).start()
    k_copy(0, 0).start()
    wq_copy(NG + 1).start()
    k_copy(1, 1).start()
    transpose_x()

    def z_body(u, c):
        wq_copy(u).wait()
        project_q(u)
        return c
    jax.lax.fori_loop(0, NG + 1, z_body, 0)
    k_copy(0, 0).wait()
    v_copy(0, 0).start()
    wo_copy(0).start()

    def a_body(n, c):
        for i in range(AC):
            scores(0, 0, n * AC + i)
        return c
    jax.lax.fori_loop(0, BB // AC, a_body, 0)
    wq_copy(NG + 1).wait()
    k_copy(1, 1).wait()
    wq_copy(NG + 2).start()
    k_copy(2, 0).start()
    step(1, 1, cd=False, zt=NG + 1)

    def body(t, c):
        zt = t + NG - (t >> HSH)
        last = (t & (HKV - 1)) == HKV - 1

        @pl.when((t & 1) == 0)
        def _():
            stream(t, 0)

            @pl.when(jnp.logical_and((t & (HKV - 1)) == HKV // 2, t < NU - HKV))
            def _():
                x_copy((t >> HSH) + 1).start()

            @pl.when((zt & (HKV - 1)) == 0)
            def _():
                x_copy(zt >> HSH).wait()
                transpose_x()
            step(t, 0, zt=zt)

        @pl.when(jnp.logical_and((t & 1) == 1, jnp.logical_not(last)))
        def _():
            stream(t, 1)
            step(t, 1, zt=zt)

            @pl.when((t & (HKV - 1)) == 1)
            def _():
                g = (t >> HSH) - 1
                for i in range(BB):
                    ost[i] = acc_s[i // CB, :, (i % CB) * SQ:(i % CB + 1) * SQ].astype(ost.dtype)
                for n in range(NCH):
                    o_copy(g, n, osem.at[n]).start()

        @pl.when(last)
        def _():
            stream(t, 1, guard_k=True)
            step(t, 1, z=False)
        return c
    jax.lax.fori_loop(2, NU, body, 0)

    v_copy(NU - 2, 0).wait()
    v_copy(NU - 1, 1).start()
    step(NU, 0, z=False, a=False)
    v_copy(NU - 1, 1).wait()
    for n in range(NCH):
        o_copy(NG - 2, n, osem.at[n]).wait()
    last_copies = [o_copy(NG - 1, n, osem.at[n]) for n in range(NCH)]
    for n in range(NCH):
        r = out_proj(HKV - 1, [attend(1, n * CB + i) for i in range(CB)]) + acc_s[n]
        for i in range(CB):
            ost[n * CB + i] = r[:, i * SQ:(i + 1) * SQ].astype(ost.dtype)
        last_copies[n].start()
    for cp in last_copies:
        cp.wait()


@jax.jit
def pallas_standalone__gqa_block_cached__near_ridge_kernel(x, k_cache, v_cache, wq, wo):
    vm = pltpu.VMEM
    dma = pltpu.SemaphoreType.DMA
    hbm = pl.BlockSpec(memory_space=pltpu.HBM)
    out_t = pl.pallas_call(
        _kernel,
        in_specs=[hbm] * 5,
        out_specs=hbm,
        out_shape=jax.ShapeDtypeStruct((B, D, SQ), x.dtype),
        scratch_shapes=[
            vm((BB, D, SQ), BF16),
            vm((BB * SQ, D), BF16),
            vm((HKV, D, W), BF16),
            vm((HKV, D, W), BF16),
            *[vm((BB, SK, DH), BF16)] * 4,
            vm((4, BB, REP * SQ, DH), BF16),
            *[vm((BB, REP * SQ, SK), F32)] * 2,
            *[vm((BB, REP * SQ, SK), BF16)] * 2,
            *[vm((BB, REP * SQ, DH), F32)] * 2,
            vm((NCH, D, CB * SQ), F32),
            vm((BB, D, SQ), BF16),
            dma(()), dma((4,)), dma(()), dma((2,)), dma((2,)), dma((NCH,)),
        ],
        compiler_params=pltpu.CompilerParams(
            vmem_limit_bytes=100 * 1024 * 1024,
            disable_bounds_checks=True,
            flags={"XLA_TPU_EVENLY_DISTRIBUTE_CRITICAL_NODES": True},
        ),
    )(jnp.transpose(x, (0, 2, 1)), k_cache, v_cache, wq, wo.T)
    return jnp.transpose(out_t, (0, 2, 1))
```
